```python
import jax
import jax.numpy as jnp

def _softmax(x, axis=-1):
    return jax.nn.softmax(x, axis=axis)

def _gelu(x):
    return jax.nn.gelu(x, approximate=True)

def _silu(x):
    return jax.nn.silu(x)

def _sigmoid(x):
    return jax.nn.sigmoid(x)

def _layernorm(x, axis=-1, eps=1e-05):
    m = jnp.mean(x, axis=axis, keepdims=True)
    v = jnp.var(x, axis=axis, keepdims=True)
    return (x - m) / jnp.sqrt(v + eps)

def _scatter_add(tgt, idx, src, axis=0):
    return tgt.at[idx].add(src)

def _segment_sum(src, seg, n):
    return jax.ops.segment_sum(src, seg, n)

class _Rng:

    def __init__(self, key):
        self._k = key

    def _next(self):
        self._k, sub = jax.random.split(self._k)
        return sub

    def normal(self, shape):
        return jax.random.normal(self._next(), shape, dtype=jnp.bfloat16)

    def randint(self, lo, hi, shape):
        return jax.random.randint(self._next(), shape, lo, hi, dtype=jnp.int32)

    def uniform(self, shape, lo=0.0, hi=1.0):
        return jax.random.uniform(self._next(), shape, jnp.bfloat16, lo, hi)

    def permutation(self, n):
        return jax.random.permutation(self._next(), n)
kernel_name = 'standalone__dilated_atrous__vision'

def setup_inputs():
    _rng = _Rng(jax.random.key(int.from_bytes(__import__("os").urandom(4), "little")))
    _w = lambda a: (lambda t: t.astype(jnp.bfloat16) if jnp.issubdtype(t.dtype, jnp.floating) else t)(jnp.asarray(a))
    H = W = 384
    C = 384
    k = 1
    return {'x': _w((lambda *s: _rng.normal(s) * 0.05)(1, H, W, C)), 'w': _w((lambda *s: _rng.normal(s) * 0.05)(k, k, C, C) * (1.0 / (k * C ** 0.5)))}

def reference(x, w):
    B, H, W, C = x.shape
    k = 1
    rate = 2
    pad = (k - 1) * rate // 2
    xp = jnp.pad(x, ((0, 0), (pad, pad), (pad, pad), (0, 0)))
    out = jnp.zeros_like(x)
    for i in range(k):
        for j in range(k):
            tap = xp[:, i * rate:i * rate + H, j * rate:j * rate + W, :].copy()
            out = out + jnp.einsum('bhwc,co->bhwo', tap, w[i, j])
    return out
```

```python
import jax
import jax.numpy as jnp
from jax import lax
import jax.experimental.pallas as pl
import jax.experimental.pallas.tpu as pltpu

_TM = 1024
_RD_ROWS = 3072
_SPR_ROWS = 128
_SPR_HALVES = 2
_N1 = 80
_WS, _WR, _WT = 6, 4096, 32
_W_BURST = 16
_W_PER_STEP = 11


@jax.jit
def pallas_standalone__dilated_atrous__vision_kernel(
    x: jax.Array,
    w: jax.Array,
):
    B, H, W, C = x.shape
    assert w.shape == (1, 1, C, C)
    M = B * H * W

    tm, rr, srows, hs, n1 = _TM, _RD_ROWS, _SPR_ROWS, _SPR_HALVES, _N1
    S, R, t = _WS, _WR, _WT
    G = M // (S * R)
    J = R // t
    NW = G * J
    NC = M // tm
    nslab = C // 128
    nspr = nslab * hs
    fill = n1 * nspr * srows
    main = M - fill
    NR = main // rr
    last = main - (NR - 1) * rr
    spr = rr // tm
    ifill = main // tm
    spg = S * R // tm
    qn = R // tm
    ilast = NC - spg
    assert G * S * R == M and J * t == R and J & (J - 1) == 0 and NC * tm == M
    assert spr * tm == rr and qn * tm == R and n1 <= ifill <= ilast
    log2_j = J.bit_length() - 1

    def kernel_function(x_hbm, w_hbm, o_hbm, buf, wbuf, rsem, wsem, fsem, osem):
        buf4 = buf.reshape(G, S, R, C)

        def read(r0, n, sem):
            return pltpu.make_async_copy(
                x_hbm.at[pl.ds(r0, n)], buf.at[pl.ds(r0, n)], sem)

        def read_main(c):
            return read(pl.multiple_of(c * rr, rr), rr, rsem.at[c])

        def read_last():
            return read((NR - 1) * rr, last, rsem.at[NR - 1])

        def write(k):
            g = lax.shift_right_logical(k, log2_j)
            off = pl.multiple_of((k & (J - 1)) * t, t)
            return pltpu.make_async_copy(
                buf4.at[g, :, pl.ds(off, t), :],
                o_hbm.at[g, :, pl.ds(off, t), :], osem)

        def start_writes(lo, hi):
            lax.fori_loop(lo, hi, lambda k, _: write(k).start(priority=1), None)

        def wait_main(i):
            c = lax.div(i, spr)

            @pl.when(jnp.logical_and(c * spr == i, c < NR - 1))
            def _():
                read_main(c).wait()

            @pl.when(i == (NR - 1) * spr)
            def _():
                read_last().wait()

        def dot(a, b):
            return jnp.dot(a, b, preferred_element_type=jnp.float32).astype(buf.dtype)

        w_copy = pltpu.make_async_copy(w_hbm, wbuf, wsem)
        w_copy.start()
        lax.fori_loop(0, NR - 1, lambda c, _: read_main(c).start(priority=1), None)
        read_last().start(priority=1)
        w_copy.wait()

        def step1(i, _):
            wait_main(i)
            r0 = pl.multiple_of(i * tm, tm)
            xv = buf[pl.ds(r0, tm), :]
            th = tm // hs
            for n in range(nslab):
                cols = slice(n * 128, (n + 1) * 128)
                res = dot(xv, wbuf[:, cols])
                for h in range(hs):
                    k = i * nspr + n * hs + h
                    read(pl.multiple_of(main + k * srows, 16), srows, fsem).start()
                    buf[pl.ds(r0 + h * th, th), cols] = res[h * th:(h + 1) * th]

        lax.fori_loop(0, n1, step1, None)

        def step2(i, issued):
            ii = jnp.maximum(i - ilast, 0)
            q = lax.div(ii, S)
            ready = jnp.minimum(lax.div(i, spg), G - 1) * J + q * (J // qn)
            r0 = jnp.where(i >= ilast, ilast * tm + (ii - q * S) * R + q * tm, i * tm)
            target = jnp.minimum(ready, _W_BURST + (i - n1) * _W_PER_STEP)
            start_writes(issued, target)
            wait_main(i)

            @pl.when(i == ifill)
            def _():
                read(main, fill, fsem).wait()

            rows = pl.ds(pl.multiple_of(r0, tm), tm)
            buf[rows, :] = dot(buf[rows, :], wbuf[...])
            return target

        issued = lax.fori_loop(n1, NC, step2, jnp.int32(0))
        start_writes(issued, NW)
        pltpu.make_async_copy(buf4, o_hbm, osem).wait()

    out = pl.pallas_call(
        kernel_function,
        in_specs=[pl.BlockSpec(memory_space=pl.ANY), pl.BlockSpec(memory_space=pl.ANY)],
        out_specs=pl.BlockSpec(memory_space=pl.ANY),
        out_shape=jax.ShapeDtypeStruct((G, S, R, C), x.dtype),
        scratch_shapes=[
            pltpu.VMEM((M, C), x.dtype),
            pltpu.VMEM((C, C), w.dtype),
            pltpu.SemaphoreType.DMA((NR,)),
            pltpu.SemaphoreType.DMA(()),
            pltpu.SemaphoreType.DMA(()),
            pltpu.SemaphoreType.DMA(()),
        ],
        compiler_params=pltpu.CompilerParams(vmem_limit_bytes=120 * 2**20),
    )(x.reshape(M, C), w.reshape(C, C))
    return out.reshape(B, H, W, C)
```

```python
import jax
import jax.numpy as jnp
from jax import lax
import jax.experimental.pallas as pl
import jax.experimental.pallas.tpu as pltpu

_TM = 1024
_N1 = 78
_BIG_ROWS = 4096
_SMALL_ROWS = 64
_PARTS = 4
_TAIL_ROWS = 768
_W_SLABS, _W_STRIDE, _W_ROWS = 6, 4096, 32
_W_FIRST = 12
_W_PER_STEP = 11


@jax.jit
def pallas_standalone__dilated_atrous__vision_kernel(
    x: jax.Array,
    w: jax.Array,
):
    B, H, W, C = x.shape
    assert w.shape == (1, 1, C, C) and C % 128 == 0
    M = B * H * W

    tm, n1, big, small, tail = _TM, _N1, _BIG_ROWS, _SMALL_ROWS, _TAIL_ROWS
    S, R, t = _W_SLABS, _W_STRIDE, _W_ROWS
    n_steps = M // tm
    n_cols = C // 128

    small_per_step = n_cols * _PARTS
    small_total = n1 * small_per_step * small
    small_base = M - small_total
    n_big = (small_base - tail - 16) // big
    first = small_base - tail - n_big * big
    first_steps = first // tm
    big_steps = big // tm
    big_waited = pl.cdiv(n1 - first_steps, big_steps)

    G = M // (S * R)
    J = R // t
    n_writes = G * J
    group_steps = S * R // tm
    slab_steps = R // tm
    last_group = n_steps - group_steps

    assert n_steps * tm == M and big_steps * tm == big and tm % (16 * _PARTS) == 0
    assert first % 16 == 0 and small % 16 == 0 and tail % 16 == 0
    assert n1 * tm <= small_base - tail and big_waited < n_big and n1 <= last_group
    assert G * S * R == M and J * t == R and J & (J - 1) == 0
    assert slab_steps * tm == R and J % slab_steps == 0
    assert _W_FIRST <= n1 // group_steps * J
    log2_j = J.bit_length() - 1

    def kernel_function(x_hbm, w_hbm, o_hbm, buf, wbuf, out_sem):
        buf4 = buf.reshape(G, S, R, C)

        def write(k):
            g = lax.shift_right_logical(k, log2_j)
            rows = pl.ds(pl.multiple_of((k & (J - 1)) * t, t), t)
            return pltpu.make_async_copy(
                buf4.at[g, :, rows, :], o_hbm.at[g, :, rows, :], out_sem)

        def start_writes(lo, hi):
            lax.fori_loop(lo, hi, lambda k, _: write(k).start(), None)

        def dot(a, b):
            return jnp.dot(a, b, preferred_element_type=jnp.float32).astype(buf.dtype)

        def read_phase(big_sems, sems):
            def read(r0, n, sem):
                return pltpu.make_async_copy(
                    x_hbm.at[pl.ds(r0, n)], buf.at[pl.ds(r0, n)], sem)

            def read_big(c):
                r0 = first + c * big
                if not isinstance(c, int):
                    r0 = pl.multiple_of(r0, 16)
                return read(r0, big, big_sems.at[c])

            w_copy = pltpu.make_async_copy(w_hbm, wbuf, sems.at[0])
            first_copy = read(0, first, sems.at[1])
            tail_copy = read(small_base - tail, tail, sems.at[2])
            small_sem = sems.at[3]

            w_copy.start()
            first_copy.start()
            lax.fori_loop(0, n_big, lambda c, _: read_big(c).start(priority=1), None)
            tail_copy.start(priority=1)
            w_copy.wait()
            first_copy.wait()

            def step(i, _):
                c = lax.div(i - first_steps, big_steps)

                @pl.when(i == first_steps + c * big_steps)
                def _():
                    read_big(c).wait()

                r0 = pl.multiple_of(i * tm, tm)
                xv = buf[pl.ds(r0, tm), :]
                part = tm // _PARTS
                for n in range(n_cols):
                    cols = slice(n * 128, (n + 1) * 128)
                    res = dot(xv, wbuf[:, cols])
                    for p in range(_PARTS):
                        k = i * small_per_step + n * _PARTS + p
                        read(pl.multiple_of(small_base + k * small, 16), small,
                             small_sem).start()
                        buf[pl.ds(r0 + p * part, part), cols] = (
                            res[p * part:(p + 1) * part])

            lax.fori_loop(0, n1, step, None)

            for c in range(big_waited, n_big):
                read_big(c).wait()
            start_writes(0, _W_FIRST)
            tail_copy.wait()
            read(small_base, small_total, small_sem).wait()

        pl.run_scoped(
            read_phase,
            pltpu.SemaphoreType.DMA((n_big,)),
            pltpu.SemaphoreType.DMA((4,)),
        )

        def step(i, started):
            ii = jnp.maximum(i - last_group, 0)
            q = lax.div(ii, S)
            r0 = jnp.where(
                i >= last_group, last_group * tm + (ii - q * S) * R + q * tm, i * tm)
            ready = (jnp.minimum(lax.div(i, group_steps), G - 1) * J
                     + q * (J // slab_steps))
            target = jnp.minimum(ready, _W_FIRST + (i - n1 + 1) * _W_PER_STEP)
            start_writes(started, target)

            rows = pl.ds(pl.multiple_of(r0, tm), tm)
            buf[rows, :] = dot(buf[rows, :], wbuf[...])
            return target

        started = lax.fori_loop(n1, n_steps, step, jnp.int32(_W_FIRST))
        start_writes(started, n_writes)
        pltpu.make_async_copy(buf4, o_hbm, out_sem).wait()

    out = pl.pallas_call(
        kernel_function,
        in_specs=[
            pl.BlockSpec(memory_space=pl.ANY),
            pl.BlockSpec(memory_space=pl.ANY),
        ],
        out_specs=pl.BlockSpec(memory_space=pl.ANY),
        out_shape=jax.ShapeDtypeStruct((G, S, R, C), x.dtype),
        scratch_shapes=[
            pltpu.VMEM((M, C), x.dtype),
            pltpu.VMEM((C, C), w.dtype),
            pltpu.SemaphoreType.DMA(()),
        ],
        compiler_params=pltpu.CompilerParams(vmem_limit_bytes=120 * 2**20),
    )(x.reshape(M, C), w.reshape(C, C))
    return out.reshape(B, H, W, C)
```

```python
import jax
import jax.numpy as jnp
from jax import lax
import jax.experimental.pallas as pl
import jax.experimental.pallas.tpu as pltpu

_TM = 1024
_N1 = 74
_BIG_ROWS = 3072
_SMALL_ROWS = 64
_STORES = (5, 5, 1)
_TAIL_ROWS = 768
_W_SLABS, _W_STRIDE, _W_ROWS = 6, 4096, 32
_W_FIRST = 12
_W_PER_STEP = 11


@jax.jit
def pallas_standalone__dilated_atrous__vision_kernel(
    x: jax.Array,
    w: jax.Array,
):
    B, H, W, C = x.shape
    assert w.shape == (1, 1, C, C) and C == 128 * len(_STORES)
    M = B * H * W

    tm, n1, big, small, tail = _TM, _N1, _BIG_ROWS, _SMALL_ROWS, _TAIL_ROWS
    S, R, t = _W_SLABS, _W_STRIDE, _W_ROWS
    n_steps = M // tm
    n_cols = C // 128

    small_per_step = n_cols + sum(_STORES)
    small_total = n1 * small_per_step * small
    small_base = M - small_total
    n_big = (small_base - tail - 16) // big
    first = small_base - tail - n_big * big
    first_steps = first // tm
    big_steps = big // tm
    big_waited = pl.cdiv(n1 - first_steps, big_steps)

    G = M // (S * R)
    J = R // t
    n_writes = G * J
    group_steps = S * R // tm
    slab_steps = R // tm
    last_group = n_steps - group_steps

    assert n_steps * tm == M and big_steps * tm == big and first_steps < big_steps
    assert first % 16 == 0 and small % 16 == 0 and tail % 16 == 0
    assert n1 * tm <= small_base - tail and big_waited < n_big and n1 <= last_group
    assert G * S * R == M and J * t == R and J & (J - 1) == 0
    assert slab_steps * tm == R and J % slab_steps == 0
    assert _W_FIRST <= n1 // group_steps * J
    log2_j = J.bit_length() - 1

    def kernel_function(x_hbm, w_hbm, o_hbm, buf, wbuf, out_sem):
        buf4 = buf.reshape(G, S, R, C)

        def write(k):
            g = lax.shift_right_logical(k, log2_j)
            rows = pl.ds(pl.multiple_of((k & (J - 1)) * t, t), t)
            return pltpu.make_async_copy(
                buf4.at[g, :, rows, :], o_hbm.at[g, :, rows, :], out_sem)

        def start_writes(lo, hi):
            lax.fori_loop(lo, hi, lambda k, _: write(k).start(), None)

        def dot(a, b):
            return jnp.dot(a, b, preferred_element_type=jnp.float32).astype(buf.dtype)

        def read_phase(big_sems, sems):
            def read(r0, n, sem):
                return pltpu.make_async_copy(
                    x_hbm.at[pl.ds(r0, n)], buf.at[pl.ds(r0, n)], sem)

            def read_big(c):
                r0 = first + c * big
                if not isinstance(c, int):
                    r0 = pl.multiple_of(r0, 16)
                return read(r0, big, big_sems.at[c])

            w_copy = pltpu.make_async_copy(w_hbm, wbuf, sems.at[0])
            first_copy = read(0, first, sems.at[1])
            tail_copy = read(small_base - tail, tail, sems.at[2])
            small_sem = sems.at[3]

            w_copy.start()
            first_copy.start()
            lax.fori_loop(0, n_big, lambda c, _: read_big(c).start(priority=1), None)
            tail_copy.start(priority=1)
            w_copy.wait()
            first_copy.wait()

            def step(i, _):
                c = lax.div(i - first_steps, big_steps)

                @pl.when(i == first_steps + c * big_steps)
                def _():
                    read_big(c).wait()

                small_ids = iter(range(small_per_step))

                def start_small():
                    k = i * small_per_step + next(small_ids)
                    read(pl.multiple_of(small_base + k * small, 16), small,
                         small_sem).start()

                r0 = pl.multiple_of(i * tm, tm)
                slabs = []
                for n in range(n_cols):
                    start_small()
                    slabs.append(buf[pl.ds(r0, tm), n * 128:(n + 1) * 128])
                xv = jnp.concatenate(slabs, axis=1)
                for n, stores in enumerate(_STORES):
                    cols = slice(n * 128, (n + 1) * 128)
                    res = dot(xv, wbuf[:, cols])
                    cuts = [p * tm // stores // 16 * 16 for p in range(stores)] + [tm]
                    for lo, hi in zip(cuts, cuts[1:]):
                        start_small()
                        buf[pl.ds(r0 + lo, hi - lo), cols] = res[lo:hi]

            lax.fori_loop(0, n1, step, None)

            for c in range(big_waited, n_big):
                read_big(c).wait()
            start_writes(0, _W_FIRST)
            tail_copy.wait()
            read(small_base, small_total, small_sem).wait()

        pl.run_scoped(
            read_phase,
            pltpu.SemaphoreType.DMA((n_big,)),
            pltpu.SemaphoreType.DMA((4,)),
        )

        def step(i, started):
            ii = jnp.maximum(i - last_group, 0)
            q = lax.div(ii, S)
            r0 = jnp.where(
                i >= last_group, last_group * tm + (ii - q * S) * R + q * tm, i * tm)
            ready = (jnp.minimum(lax.div(i, group_steps), G - 1) * J
                     + q * (J // slab_steps))
            target = jnp.minimum(ready, _W_FIRST + (i - n1 + 1) * _W_PER_STEP)
            start_writes(started, target)

            rows = pl.ds(pl.multiple_of(r0, tm), tm)
            buf[rows, :] = dot(buf[rows, :], wbuf[...])
            return target

        started = lax.fori_loop(n1, n_steps, step, jnp.int32(_W_FIRST))
        start_writes(started, n_writes)
        pltpu.make_async_copy(buf4, o_hbm, out_sem).wait()

    out = pl.pallas_call(
        kernel_function,
        in_specs=[
            pl.BlockSpec(memory_space=pl.ANY),
            pl.BlockSpec(memory_space=pl.ANY),
        ],
        out_specs=pl.BlockSpec(memory_space=pl.ANY),
        out_shape=jax.ShapeDtypeStruct((G, S, R, C), x.dtype),
        scratch_shapes=[
            pltpu.VMEM((M, C), x.dtype),
            pltpu.VMEM((C, C), w.dtype),
            pltpu.SemaphoreType.DMA(()),
        ],
        compiler_params=pltpu.CompilerParams(vmem_limit_bytes=120 * 2**20),
    )(x.reshape(M, C), w.reshape(C, C))
    return out.reshape(B, H, W, C)
```

```python
import jax
import jax.numpy as jnp
from jax import lax
import jax.experimental.pallas as pl
import jax.experimental.pallas.tpu as pltpu

_SLAB = 4096
_TM = 1024
_N1 = 74
_SMALL = 64
_STORES = (5, 5, 1)
_TAIL = 768
_W_SLABS = 6
_W_ROWS = 32
_W_FIRST = 12
_W_PER_STEP = 11


def _split(i, n):
    assert n & (n - 1) == 0
    return lax.shift_right_logical(i, n.bit_length() - 1), i & (n - 1)


@jax.jit
def pallas_standalone__dilated_atrous__vision_kernel(
    x: jax.Array,
    w: jax.Array,
):
    B, H, W, C = x.shape
    assert w.shape == (1, 1, C, C) and C == 128 * len(_STORES)
    M = B * H * W
    n_slabs = M // _SLAB
    n_steps = M // _TM
    slab_steps = _SLAB // _TM
    assert n_slabs * _SLAB == M and slab_steps * _TM == _SLAB

    small_per_step = len(_STORES) + sum(_STORES)
    small_base = M - _N1 * small_per_step * _SMALL
    n_big, small_row = divmod(small_base, _SLAB)
    last = small_row - _TAIL
    assert last > 0 and last % 16 == 0 and small_base % _SMALL == 0
    assert n_big + 1 < n_slabs
    assert pl.cdiv(_N1, slab_steps) == n_big

    n_groups = n_slabs // _W_SLABS
    group_writes = _SLAB // _W_ROWS
    n_writes = n_groups * group_writes
    group_steps = _W_SLABS * slab_steps
    last_group = n_steps - group_steps
    assert n_groups * _W_SLABS == n_slabs and group_writes % slab_steps == 0
    assert _N1 <= last_group and _W_FIRST <= _N1 // group_steps * group_writes

    def kernel_function(x_hbm, w_hbm, o_hbm, buf, wbuf, out_sem):
        def write(k):
            g, j = _split(k, group_writes)
            slabs = pl.ds(g * _W_SLABS, _W_SLABS)
            rows = pl.ds(pl.multiple_of(j * _W_ROWS, _W_ROWS), _W_ROWS)
            return pltpu.make_async_copy(
                buf.at[slabs, rows], o_hbm.at[slabs, rows], out_sem)

        def start_writes(lo, hi):
            lax.fori_loop(lo, hi, lambda k, _: write(k).start(), None)

        def dot(a, b):
            return jnp.dot(a, b, preferred_element_type=jnp.float32).astype(buf.dtype)

        def read_phase(big_sems, sems):
            def read(idx, sem):
                return pltpu.make_async_copy(x_hbm.at[idx], buf.at[idx], sem)

            def read_big(s):
                return read(s, big_sems.at[s])

            def read_small(k):
                s, r = _split(small_base + k * _SMALL, _SLAB)
                rows = pl.ds(pl.multiple_of(r, _SMALL), _SMALL)
                return read((s, rows), sems.at[jnp.where(s == n_big, 3, 4)])

            w_copy = pltpu.make_async_copy(w_hbm, wbuf, sems.at[0])
            last_copy = read((n_big, pl.ds(0, last)), sems.at[1])
            tail_copy = read((n_big, pl.ds(last, _TAIL)), sems.at[2])

            w_copy.start()
            lax.fori_loop(
                0, n_big, lambda s, _: read_big(s).start(priority=1), None)
            last_copy.start(priority=1)
            w_copy.wait()
            tail_copy.start(priority=1)

            def step(i, _):
                s, q = _split(i, slab_steps)

                @pl.when(q == 0)
                def _():
                    read_big(s).wait()

                small_ids = iter(range(small_per_step))

                def start_small():
                    read_small(i * small_per_step + next(small_ids)).start()

                r0 = pl.multiple_of(q * _TM, _TM)
                blocks = []
                for n in range(len(_STORES)):
                    start_small()
                    blocks.append(buf[s, pl.ds(r0, _TM), n * 128:(n + 1) * 128])
                xv = jnp.concatenate(blocks, axis=1)
                for n, stores in enumerate(_STORES):
                    cols = slice(n * 128, (n + 1) * 128)
                    res = dot(xv, wbuf[:, cols])
                    cuts = [p * _TM // stores // 16 * 16 for p in range(stores + 1)]
                    for lo, hi in zip(cuts, cuts[1:]):
                        start_small()
                        buf[s, pl.ds(r0 + lo, hi - lo), cols] = res[lo:hi]

            lax.fori_loop(0, _N1, step, None)

            last_copy.wait()
            start_writes(0, _W_FIRST)
            tail_copy.wait()
            read((n_big, pl.ds(small_row, _SLAB - small_row)), sems.at[3]).wait()
            read(pl.ds(n_big + 1, n_slabs - n_big - 1), sems.at[4]).wait()

        pl.run_scoped(
            read_phase,
            pltpu.SemaphoreType.DMA((n_big,)),
            pltpu.SemaphoreType.DMA((5,)),
        )

        def step(i, started):
            s, q = _split(i, slab_steps)
            ii = jnp.maximum(i - last_group, 0)
            rounds = lax.div(ii, _W_SLABS)
            in_last = i >= last_group
            s = jnp.where(in_last, n_slabs - _W_SLABS + ii - rounds * _W_SLABS, s)
            q = jnp.where(in_last, rounds, q)
            ready = (jnp.minimum(lax.div(i, group_steps), n_groups - 1) * group_writes
                     + rounds * (group_writes // slab_steps))
            target = jnp.minimum(ready, _W_FIRST + (i - _N1 + 1) * _W_PER_STEP)
            start_writes(started, target)

            rows = pl.ds(pl.multiple_of(q * _TM, _TM), _TM)
            buf[s, rows, :] = dot(buf[s, rows, :], wbuf[...])
            return target

        started = lax.fori_loop(_N1, n_steps, step, jnp.int32(_W_FIRST))
        start_writes(started, n_writes)
        pltpu.make_async_copy(buf, o_hbm, out_sem).wait()

    out = pl.pallas_call(
        kernel_function,
        in_specs=[
            pl.BlockSpec(memory_space=pl.ANY),
            pl.BlockSpec(memory_space=pl.ANY),
        ],
        out_specs=pl.BlockSpec(memory_space=pl.ANY),
        out_shape=jax.ShapeDtypeStruct((n_slabs, _SLAB, C), x.dtype),
        scratch_shapes=[
            pltpu.VMEM((n_slabs, _SLAB, C), x.dtype),
            pltpu.VMEM((C, C), w.dtype),
            pltpu.SemaphoreType.DMA(()),
        ],
        compiler_params=pltpu.CompilerParams(vmem_limit_bytes=120 * 2**20),
    )(x.reshape(n_slabs, _SLAB, C), w.reshape(C, C))
    return out.reshape(B, H, W, C)
```
